```python
import os as _os
_os.environ.setdefault("JAX_PLATFORMS", "cpu")
import jax
import jax.numpy as jnp

def _softmax(x, axis=-1):
    return jax.nn.softmax(x, axis=axis)
def _gelu(x):
    return jax.nn.gelu(x, approximate=True)
def _silu(x):
    return jax.nn.silu(x)
def _sigmoid(x):
    return jax.nn.sigmoid(x)
def _layernorm(x, axis=-1, eps=1e-5):
    m = jnp.mean(x, axis=axis, keepdims=True)
    v = jnp.var(x, axis=axis, keepdims=True)
    return (x - m) / jnp.sqrt(v + eps)
def _scatter_add(tgt, idx, src, axis=0):
    return tgt.at[idx].add(src)
def _segment_sum(src, seg, n):
    return jax.ops.segment_sum(src, seg, n)
class _Rng:
    def __init__(self, key):
        self._k = key
    def _next(self):
        self._k, sub = jax.random.split(self._k)
        return sub
    def normal(self, shape):
        return jax.random.normal(self._next(), shape, dtype=jnp.bfloat16)
    def randint(self, lo, hi, shape):
        return jax.random.randint(self._next(), shape, lo, hi, dtype=jnp.int32)
    def uniform(self, shape, lo=0.0, hi=1.0):
        return jax.random.uniform(self._next(), shape, jnp.bfloat16, lo, hi)
    def permutation(self, n):
        return jax.random.permutation(self._next(), n)


kernel_name = 'standalone__mha_block_cached__near_ridge'

def setup_inputs():
    _rng = _Rng(jax.random.key(int.from_bytes(__import__("os").urandom(4), "little")))
    _w = (lambda a: (lambda t: t.astype(jnp.bfloat16) if jnp.issubdtype(t.dtype, jnp.floating) else t)(jnp.asarray(a)))
    B, Sq, D = 16, 64, 576
    H, Sk, Dh = 32, 64, 128
    return {
        "x": _w((lambda *s: _rng.normal(s) * 0.8)(B, Sq, D)),
        "k_cache": _w((lambda *s: _rng.normal(s) * 0.8)(B, H, Sk, Dh)),
        "v_cache": _w((lambda *s: _rng.normal(s) * 0.05)(B, H, Sk, Dh)),
        "wq": _w((lambda *s: _rng.normal(s) * 0.8)(D, H * Dh) * (D ** -0.5)),
        "wo": _w((lambda *s: _rng.normal(s) * 0.05)(H * Dh, D) * ((H * Dh) ** -0.5)),
    }

def reference(x, k_cache, v_cache, wq, wo):
    B, Sq, D = x.shape
    H, Dh = 32, 128
    q = (lambda x, *d: x.transpose(*d))((x @ wq).reshape(B, Sq, H, Dh), 0, 2, 1, 3)
    scores = jnp.einsum("bhqd,bhkd->bhqk", q, k_cache) * (Dh ** -0.5)
    p = _softmax(scores, axis=-1)
    o = jnp.einsum("bhqk,bhkd->bhqd", p, v_cache)
    return (lambda x, *d: x.transpose(*d))(o, 0, 2, 1, 3).reshape(B, Sq, H * Dh) @ wo
```

```python
import functools

import jax
import jax.numpy as jnp
import jax.experimental.pallas as pl
import jax.experimental.pallas.tpu as pltpu

_LOG2E = 1.4426950408889634


def _mha_kernel(x_ref, k_ref, v_ref, wq_ref, wo_ref, o_ref, q_scr, o_scr, acc_scr,
                *, G, NP, scale):
    g = pl.program_id(0)

    q = jnp.dot(x_ref[...], wq_ref[...], preferred_element_type=jnp.float32)
    q_scr[...] = q.astype(jnp.bfloat16)

    row = jax.lax.broadcasted_iota(jnp.int32, (128, 128), 0)
    col = jax.lax.broadcasted_iota(jnp.int32, (128, 128), 1)
    valid = (row < 64) == (col < 64)
    c = scale * _LOG2E

    for p in range(NP):
        for h in range(G):
            qt = q_scr[p * 128:(p + 1) * 128, h * 128:(h + 1) * 128]
            kt = k_ref[2 * p:2 * p + 2, h].reshape(128, 128)
            vt = v_ref[2 * p:2 * p + 2, h].reshape(128, 128)
            s = jax.lax.dot_general(qt, kt, (((1,), (1,)), ((), ())),
                                    preferred_element_type=jnp.float32)
            s = jnp.where(valid, s, -jnp.inf)
            m = jnp.max(s, axis=-1, keepdims=True)
            e = jnp.exp2((s - m) * c)
            l = jnp.sum(e, axis=-1, keepdims=True)
            pr = (e * pl.reciprocal(l, approx=False)).astype(jnp.bfloat16)
            o = jnp.dot(pr, vt, preferred_element_type=jnp.float32)
            o_scr[p * 128:(p + 1) * 128, h * 128:(h + 1) * 128] = o.astype(jnp.bfloat16)

    contrib = jnp.dot(o_scr[...], wo_ref[...], preferred_element_type=jnp.float32)

    @pl.when(g == 0)
    def _():
        acc_scr[...] = contrib

    @pl.when(g > 0)
    def _():
        acc_scr[...] += contrib

    @pl.when(g == pl.num_programs(0) - 1)
    def _():
        o_ref[...] = acc_scr[...].astype(o_ref.dtype)


@jax.jit
def pallas_standalone__mha_block_cached__near_ridge_kernel(x, k_cache, v_cache, wq, wo):
    B, Sq, D = x.shape
    _, H, Sk, Dh = k_cache.shape
    G = 4
    M = B * Sq
    NP = B // 2
    x2 = x.reshape(M, D)
    kernel = functools.partial(_mha_kernel, G=G, NP=NP, scale=Dh ** -0.5)
    out = pl.pallas_call(
        kernel,
        grid=(H // G,),
        in_specs=[
            pl.BlockSpec((M, D), lambda g: (0, 0)),
            pl.BlockSpec((B, G, Sk, Dh), lambda g: (0, g, 0, 0)),
            pl.BlockSpec((B, G, Sk, Dh), lambda g: (0, g, 0, 0)),
            pl.BlockSpec((D, G * Dh), lambda g: (0, g)),
            pl.BlockSpec((G * Dh, D), lambda g: (g, 0)),
        ],
        out_specs=pl.BlockSpec((M, D), lambda g: (0, 0)),
        out_shape=jax.ShapeDtypeStruct((M, D), x.dtype),
        scratch_shapes=[
            pltpu.VMEM((M, G * Dh), jnp.bfloat16),
            pltpu.VMEM((M, G * Dh), jnp.bfloat16),
            pltpu.VMEM((M, D), jnp.float32),
        ],
        compiler_params=pltpu.CompilerParams(
            dimension_semantics=("arbitrary",),
            vmem_limit_bytes=100 * 1024 * 1024,
        ),
    )(x2, k_cache, v_cache, wq, wo)
    return out.reshape(B, Sq, D)
```

```python
import functools

import jax
import jax.numpy as jnp
import jax.experimental.pallas as pl
import jax.experimental.pallas.tpu as pltpu

_LOG2E = 1.4426950408889634
_NT = (((1,), (1,)), ((), ()))
_TN = (((0,), (0,)), ((), ()))

_G = 4
_CH = 2
_QPER = 3
_APER = 2
_AIT = 2


def _softmax_tile(qt, kt, c):
    st = jax.lax.dot_general(kt, qt, _NT, preferred_element_type=jnp.float32)
    lo = jax.lax.broadcasted_iota(jnp.int32, (64, 128), 1) < 64
    t = jnp.where(lo, st[:64], st[64:])
    m = jnp.max(t, axis=0, keepdims=True)
    e = jnp.exp2((t - m) * c)
    l = jnp.sum(e, axis=0, keepdims=True)
    return e * pl.reciprocal(l, approx=True)


def _pv_tile(pn, vt):
    lo = jax.lax.broadcasted_iota(jnp.int32, (64, 128), 1) < 64
    z = jnp.zeros_like(pn)
    pt = jnp.concatenate([jnp.where(lo, pn, z), jnp.where(lo, z, pn)], axis=0).astype(jnp.bfloat16)
    return jax.lax.dot_general(pt, vt, _TN, preferred_element_type=jnp.float32)


def _attn_order(units):
    n = len(units)
    seq = [('S', units[0]), ('S', units[1]), ('PV', units[0])]
    for u in range(1, n - 1):
        seq += [('S', units[u + 1]), ('O', units[u - 1]), ('PV', units[u])]
    seq += [('PV', units[n - 1]), ('O', units[n - 2]), ('O', units[n - 1])]
    return seq


def _mha_kernel(x_hbm, k_hbm, v_hbm, wq_hbm, wot_hbm, out_hbm,
                x_v, k_v, v_v, wq_v, wot_v, q_scr, o_scr, acc_scr, acct_scr, out_v, sems,
                *, H, NP, scale):
    G, CH = _G, _CH
    c = scale * _LOG2E
    R = CH * 128
    NC = NP // CH
    NG = H // G
    GW = G * 128
    D = out_v.shape[1]
    DM = (D // 128) * 128
    QIT = (NG - 2) // _QPER
    NLOOPG = _APER * _AIT

    kvw = lambda gs: [(n, g) for g in gs for n in ('k', 'v', 'wot')]
    groups = [
        [('wq', 0), ('x', 0)],
        [('x', 1), ('x', 2)],
        [('x', 3), ('wq', 1)],
        [('wq', g) for g in range(2, NG)],
        kvw(range(0, NLOOPG)),
        kvw(range(NLOOPG, NG)),
    ]
    sem_of = {key: i for i, grp in enumerate(groups) for key in grp}
    out_sem = len(groups)

    def cp(key):
        kind, i = key
        if kind == 'x':
            sl = (slice(i * R, (i + 1) * R), slice(None))
            return pltpu.make_async_copy(x_hbm.at[sl], x_v.at[sl], sems.at[sem_of[key]])
        if kind in ('wq', 'wot'):
            src, dst = (wq_hbm, wq_v) if kind == 'wq' else (wot_hbm, wot_v)
            sl = (slice(None), slice(i * GW, (i + 1) * GW))
            return pltpu.make_async_copy(src.at[sl], dst.at[sl], sems.at[sem_of[key]])
        if kind in ('k', 'v'):
            src, dst = (k_hbm, k_v) if kind == 'k' else (v_hbm, v_v)
            sl = (slice(None), slice(i * G, (i + 1) * G))
            return pltpu.make_async_copy(src.at[sl], dst.at[sl], sems.at[sem_of[key]])
        r0, r1 = i
        return pltpu.make_async_copy(out_v.at[r0:r1, :], out_hbm.at[r0:r1, :], sems.at[out_sem])

    def fence(i):
        for key in groups[i]:
            cp(key).wait()

    def cols(g, w=GW, extra=0):
        if isinstance(g, int):
            return slice(g * GW + extra, g * GW + extra + w)
        return pl.ds(pl.multiple_of(g * GW + extra, 128), w)

    outs = []

    def qproj(g, ci):
        q = jnp.dot(x_v[ci * R:(ci + 1) * R, :], wq_v[:, cols(g)], preferred_element_type=jnp.float32)
        q_scr[ci * R:(ci + 1) * R, cols(g)] = q.astype(jnp.bfloat16)

    def run_attn(gmap, final_g):
        pn = {}

        def is_final(slot):
            return isinstance(gmap[slot], int) and gmap[slot] == final_g

        def smax(slot, ci):
            g = gmap[slot]
            for p in range(ci * CH, (ci + 1) * CH):
                for h in range(G):
                    qt = q_scr[p * 128:(p + 1) * 128, cols(g, 128, h * 128)]
                    kt = k_v[2 * p:2 * p + 2, g * G + h].reshape(128, 128)
                    pn[slot, p, h] = _softmax_tile(qt, kt, c)

        def pv(slot, ci):
            g = gmap[slot]
            for p in range(ci * CH, (ci + 1) * CH):
                for h in range(G):
                    vt = v_v[2 * p:2 * p + 2, g * G + h].reshape(128, 128)
                    o = _pv_tile(pn.pop((slot, p, h)), vt)
                    o_scr[p * 128:(p + 1) * 128, cols(slot, 128, h * 128)] = o.astype(jnp.bfloat16)

        def oproj_rows(slot, r0, r1):
            g = gmap[slot]
            final = is_final(slot)
            rows = slice(r0, r1)
            oc = o_scr[rows, cols(slot)]

            def main(n):
                nc = slice(n * 128, (n + 1) * 128)
                m = jax.lax.dot_general(oc, wot_v[nc, cols(g)], _NT, preferred_element_type=jnp.float32)
                if final:
                    out_v[rows, nc] = (acc_scr[rows, nc] + m).astype(jnp.bfloat16)
                else:
                    acc_scr[rows, nc] += m

            def tail(pi):
                pr = slice(r0 + pi * 128, r0 + (pi + 1) * 128)
                t = jax.lax.dot_general(wot_v[DM:D, cols(g)], o_scr[pr, cols(slot)], _NT,
                                        preferred_element_type=jnp.float32)
                if final:
                    out_v[pr, DM:D] = (acct_scr[:, pr] + t).T.astype(jnp.bfloat16)
                else:
                    acct_scr[:, pr] += t

            for n in range(DM // 128):
                main(n)
                if n < (r1 - r0) // 128:
                    tail(n)
            if final:
                d = cp(('out', (r0, r1)))
                d.start()
                outs.append(d)

        def oproj(slot, ci):
            if is_final(slot) and ci == NC - 1:
                for r0 in range(ci * R, (ci + 1) * R, 128):
                    oproj_rows(slot, r0, r0 + 128)
            else:
                oproj_rows(slot, ci * R, (ci + 1) * R)

        fns = {'S': smax, 'PV': pv, 'O': oproj}
        units = [(s, ci) for s in range(len(gmap)) for ci in range(NC)]
        for name, unit in _attn_order(units):
            fns[name](*unit)

    for grp in groups:
        for key in grp:
            cp(key).start()
    acc_scr[...] = jnp.zeros_like(acc_scr)
    acct_scr[...] = jnp.zeros_like(acct_scr)

    fence(0)
    qproj(0, 0)
    fence(1)
    qproj(0, 1)
    qproj(0, 2)
    fence(2)
    qproj(0, 3)
    for ci in range(NC):
        qproj(1, ci)
    fence(3)

    def qbody(i, carry):
        for gg in range(_QPER):
            for ci in range(NC):
                qproj(2 + i * _QPER + gg, ci)
        return carry

    jax.lax.fori_loop(0, QIT, qbody, 0)
    fence(4)

    def abody(i, carry):
        run_attn([i * _APER + s for s in range(_APER)], None)
        return carry

    jax.lax.fori_loop(0, _AIT, abody, 0)
    fence(5)
    run_attn(list(range(NLOOPG, NG)), NG - 1)
    for d in outs:
        d.wait()


@jax.jit
def pallas_standalone__mha_block_cached__near_ridge_kernel(x, k_cache, v_cache, wq, wo):
    B, Sq, D = x.shape
    _, H, Sk, Dh = k_cache.shape
    assert Sq == 64 and Sk == 64 and Dh == 128 and B == 16 and H == 32
    M = B * Sq
    DM = (D // 128) * 128
    bf = jnp.bfloat16
    kernel = functools.partial(_mha_kernel, H=H, NP=B // 2, scale=Dh ** -0.5)
    out = pl.pallas_call(
        kernel,
        in_specs=[pl.BlockSpec(memory_space=pl.ANY)] * 5,
        out_specs=pl.BlockSpec(memory_space=pl.ANY),
        out_shape=jax.ShapeDtypeStruct((M, D), x.dtype),
        scratch_shapes=[
            pltpu.VMEM((M, D), bf),
            pltpu.VMEM((B, H, Sk, Dh), bf),
            pltpu.VMEM((B, H, Sk, Dh), bf),
            pltpu.VMEM((D, H * Dh), bf),
            pltpu.VMEM((D, H * Dh), bf),
            pltpu.VMEM((M, H * Dh), bf),
            pltpu.VMEM((M, (H // _G - _APER * _AIT) * _G * Dh), bf),
            pltpu.VMEM((M, DM), jnp.float32),
            pltpu.VMEM((D - DM, M), jnp.float32),
            pltpu.VMEM((M, D), bf),
            pltpu.SemaphoreType.DMA((7,)),
        ],
        compiler_params=pltpu.CompilerParams(vmem_limit_bytes=100 * 1024 * 1024),
    )(x.reshape(M, D), k_cache, v_cache, wq, wo.T)
    return out.reshape(B, Sq, D)
```

```python
import functools

import jax
import jax.numpy as jnp
import jax.experimental.pallas as pl
import jax.experimental.pallas.tpu as pltpu

_LOG2E = 1.4426950408889634
_NT = (((1,), (1,)), ((), ()))
_TN = (((0,), (0,)), ((), ()))

_G = 4
_CH = 2
_BODY = 12
_NIT = 2
_STAGES = ((256, 256), (512, 384), (768, 640), (1024, 1664), (1024, 3584))
_ORDER = ("s3,T1,m3,p3,p4,m2,s0,t0,p1,T0,s2,p7,p6,x2,m0,s1,x3,x4,p2,x7,x6,x0,p0,x1,t1,m1,p5,x5"
          ).split(",")


def _ld(ref, r0, r1, cs):
    return pltpu.bitcast(ref[r0 // 2:r1 // 2, cs], jnp.bfloat16)


def _st(ref, r0, r1, cs, val):
    ref[r0 // 2:r1 // 2, cs] = pltpu.bitcast(val, jnp.uint32)


def _lo_mask():
    return jax.lax.broadcasted_iota(jnp.int32, (64, 128), 1) < 64


def _softmax_cols(t, c):
    m = jnp.max(t, axis=0, keepdims=True)
    e = jnp.exp2((t - m) * c)
    l = jnp.sum(e, axis=0, keepdims=True)
    return e * (1.0 / l)


def _mha_kernel(x_hbm, k_hbm, v_hbm, wq_hbm, wot_hbm, out_hbm,
                x_v, k_v, v_v, wq_v, wot_v, q_scr, o_scr, w2_scr, sd_c, m2_c, pn_c,
                acc_scr, acct_scr, out_v, sems, *, H, NP, scale):
    G, CH = _G, _CH
    c = scale * _LOG2E
    R = CH * 128
    NC = NP // CH
    NG = H // G
    NU = NG * NC
    GW = G * 128
    D = out_v.shape[1]
    DM = (D // 128) * 128
    GB = _BODY // NC

    groups = _dma_groups(H, NG, GB)
    loop_sem0 = len(_STAGES)
    final_sem = len(groups) - 1
    out_sem = len(groups)
    sem_of = {key: i for i, grp in enumerate(groups) for key in grp}

    def dsl(i, w):
        if isinstance(i, int):
            return slice(i * w, (i + 1) * w)
        return pl.ds(pl.multiple_of(i * w, w), w)

    def cp(key, sem=None):
        kind, i = key
        if kind == 'out':
            return pltpu.make_async_copy(out_v.at[i[0]:i[1], :], out_hbm.at[i[0]:i[1], :], sems.at[out_sem])
        if sem is None:
            sem = sems.at[sem_of[key]]
        if kind == 'x':
            src, dst, sl = x_hbm, x_v, (slice(i[0], i[1]), slice(0, DM))
        elif kind == 'xt':
            src, dst, sl = x_hbm, x_v, (slice(None), slice(DM, D))
        elif kind == 'wq':
            src, dst, sl = wq_hbm, wq_v, (slice(0, DM), slice(i[0], i[1]))
        elif kind == 'wqt':
            src, dst, sl = wq_hbm, wq_v, (slice(DM, D), slice(None))
        elif kind == 'wot':
            src, dst, sl = wot_hbm, wot_v, (slice(None), dsl(i, GW))
        else:
            src, dst = (k_hbm, k_v) if kind == 'k' else (v_hbm, v_v)
            sl = (slice(None), dsl(i, G))
        return pltpu.make_async_copy(src.at[sl], dst.at[sl], sem)

    def fence(i):
        for key in groups[i]:
            cp(key).wait()

    def cols(g, w=GW, extra=0):
        if isinstance(g, int):
            return slice(g * GW + extra, g * GW + extra + w)
        return pl.ds(pl.multiple_of(g * GW + extra, 128), w)

    outs = []

    def qblock(r0, r1, c0, c1):
        q = jnp.dot(x_v[r0:r1, 0:DM], wq_v[0:DM, c0:c1], preferred_element_type=jnp.float32)
        _st(q_scr, r0, r1, slice(c0, c1), q.astype(jnp.bfloat16))

    def qblocks(r0, r1, c0, c1):
        return [functools.partial(qblock, ra, min(ra + R, r1), ca, min(ca + GW, c1))
                for ca in range(c0, c1, GW) for ra in range(r0, r1, R)]

    def build_w2():
        for p in range(NP):
            xt = x_v[p * 128:(p + 1) * 128, DM:D]
            z = jnp.zeros((64, 64), xt.dtype)
            top = jnp.concatenate([z, xt[:64]], axis=1)
            bot = jnp.concatenate([xt[64:], z], axis=1)
            _st(w2_scr, p * 128, (p + 1) * 128, slice(None), jnp.concatenate([top, bot], axis=0))

    class Pipe:
        def __init__(self, gb):
            self.gb = gb
            self.sd, self.m2, self.tt, self.pn = {}, {}, {}, {}

        def grp(self, r):
            return self.gb + r // NC

        def tiles(self, r):
            ci = r % NC
            return [(r, p, h) for p in range(ci * CH, (ci + 1) * CH) for h in range(G)]

        def s_tile(self, r, p, h):
            g = self.grp(r)
            lo = _lo_mask()
            hc = cols(g, 128, h * 128)
            q1 = _ld(q_scr, p * 128, p * 128 + 64, hc)
            q2 = _ld(q_scr, p * 128 + 64, (p + 1) * 128, hc)
            wt = wq_v[DM:D, hc]
            k1 = k_v[2 * p, g * G + h]
            k2 = k_v[2 * p + 1, g * G + h]
            oa = jax.lax.dot_general(k1, jnp.concatenate([q1, wt], axis=0), _NT,
                                     preferred_element_type=jnp.float32)
            ob = jax.lax.dot_general(k2, jnp.concatenate([wt, q2], axis=0), _NT,
                                     preferred_element_type=jnp.float32)
            self.sd[r, p, h] = jnp.where(lo, oa, ob)
            self.m2[r, p, h] = jnp.where(lo, ob, oa).astype(jnp.bfloat16)

        def t_mm(self, r, pi):
            p = (r % NC) * CH + pi
            mc = jnp.concatenate([self.m2.pop((r, p, h)) for h in range(G)], axis=0)
            t = jax.lax.dot_general(mc, _ld(w2_scr, p * 128, (p + 1) * 128, slice(None)), _NT,
                                    preferred_element_type=jnp.float32)
            for h in range(G):
                self.tt[r, p, h] = t[h * 64:(h + 1) * 64]

        def sm_tile(self, r, p, h):
            self.pn[r, p, h] = _softmax_cols(self.sd.pop((r, p, h)) + self.tt.pop((r, p, h)), c)

        def pv_tile(self, r, p, h):
            g = self.grp(r)
            lo = _lo_mask()
            pn = self.pn.pop((r, p, h))
            z = jnp.zeros_like(pn)
            pt = jnp.concatenate([jnp.where(lo, pn, z), jnp.where(lo, z, pn)], axis=0).astype(jnp.bfloat16)
            vt = v_v[2 * p:2 * p + 2, g * G + h].reshape(128, 128)
            o = jax.lax.dot_general(pt, vt, _TN, preferred_element_type=jnp.float32)
            slot = (r // NC) % GB
            _st(o_scr, p * 128, (p + 1) * 128, cols(slot, 128, h * 128), o.astype(jnp.bfloat16))

        def o_parts(self, r, r0, r1):
            g = self.grp(r)
            final = isinstance(g, int) and g == NG - 1
            slot = (r // NC) % GB
            rows = slice(r0, r1)

            def main(n):
                nc = slice(n * 128, (n + 1) * 128)
                m = jax.lax.dot_general(_ld(o_scr, r0, r1, cols(slot)), wot_v[nc, cols(g)], _NT,
                                        preferred_element_type=jnp.float32)
                if final:
                    out_v[rows, nc] = (acc_scr[rows, nc] + m).astype(jnp.bfloat16)
                else:
                    acc_scr[rows, nc] += m

            def tail(pi):
                a, b = r0 + pi * 128, r0 + (pi + 1) * 128
                t = jax.lax.dot_general(wot_v[DM:D, cols(g)], _ld(o_scr, a, b, cols(slot)), _NT,
                                        preferred_element_type=jnp.float32)
                if final:
                    out_v[a:b, DM:D] = (acct_scr[:, a:b] + t).T.astype(jnp.bfloat16)
                else:
                    acct_scr[:, a:b] += t

            def write_out():
                d = cp(('out', (r0, r1)))
                d.start()
                outs.append(d)

            mains = [functools.partial(main, n) for n in range(DM // 128)]
            tails = [functools.partial(tail, i) for i in range((r1 - r0) // 128)]
            return mains, tails, (write_out if final else None)

        def prologue(self, fill):
            fill = list(fill)

            def f():
                if fill:
                    fill.pop(0)()

            for u in (0, 1):
                for tl in self.tiles(u):
                    self.s_tile(*tl)
                f()
            for u in (0, 1):
                for pi in range(CH):
                    self.t_mm(u, pi)
                for tl in self.tiles(u):
                    self.sm_tile(*tl)
                f()
                if u == 0:
                    for tl in self.tiles(2):
                        self.s_tile(*tl)
                    f()
            for tl in self.tiles(0):
                self.pv_tile(*tl)
            while fill:
                f()

        def step(self, k, nr, pre=()):
            for f in pre:
                f()
            ci = (k - 1) % NC
            g = self.grp(k - 1)
            if isinstance(g, int) and g == NG - 1 and ci == NC - 1:
                for r0 in range(ci * R, (ci + 1) * R, 128):
                    mains, tails, write_out = self.o_parts(k - 1, r0, r0 + 128)
                    for f in tails + mains:
                        f()
                    write_out()
                return
            mains, tails, write_out = self.o_parts(k - 1, ci * R, (ci + 1) * R)
            omap = {f'm{i}': m for i, m in enumerate(mains)}
            omap.update({f't{i}': t for i, t in enumerate(tails)})
            left = len(omap)
            for tok in _ORDER:
                i = int(tok[1:])
                if tok in omap:
                    omap[tok]()
                    left -= 1
                    if left == 0 and write_out is not None:
                        write_out()
                elif tok[0] == 's' and k + 2 < nr:
                    for tl in self.tiles(k + 2)[2 * i:2 * i + 2]:
                        self.s_tile(*tl)
                elif tok[0] == 'T' and k + 1 < nr:
                    self.t_mm(k + 1, i)
                elif tok[0] == 'x' and k + 1 < nr:
                    self.sm_tile(*self.tiles(k + 1)[i])
                elif tok[0] == 'p' and k < nr:
                    self.pv_tile(*self.tiles(k)[i])

        def save(self, k):
            for i, tl in enumerate(self.tiles(k + 1)):
                sd_c[i] = self.sd.pop(tl)
                m2_c[i] = pltpu.bitcast(self.m2.pop(tl), jnp.uint32)
            for i, tl in enumerate(self.tiles(k)):
                pn_c[i] = self.pn.pop(tl)

        def restore(self, k):
            for i, tl in enumerate(self.tiles(k + 1)):
                self.sd[tl] = sd_c[i]
                self.m2[tl] = pltpu.bitcast(m2_c[i], jnp.bfloat16)
            for i, tl in enumerate(self.tiles(k)):
                self.pn[tl] = pn_c[i]

    for grp in groups:
        for key in grp:
            cp(key).start()
    acc_scr[...] = jnp.zeros_like(acc_scr)
    acct_scr[...] = jnp.zeros_like(acct_scr)

    pr, pc = 0, 0
    for si, (r1, c1) in enumerate(_STAGES):
        fence(si)
        qs = qblocks(pr, r1, 0, c1) + qblocks(0, pr, pc, c1)
        if si < len(_STAGES) - 1:
            for f in qs:
                f()
        pr, pc = r1, c1
    build_w2()
    nfill = 6
    for f in qs[:-nfill]:
        f()
    pipe = Pipe(0)
    pipe.prologue(qs[-nfill:])
    pipe.save(1)

    def body(i, carry):
        for kind, gi in groups[loop_sem0]:
            cp((kind, gi + i * GB), sems.at[loop_sem0 + i]).wait()
        p = Pipe(i * GB)
        p.restore(1)
        for k in range(1, _BODY + 1):
            p.step(k, NU + 2)
        p.save(_BODY + 1)
        return carry

    jax.lax.fori_loop(0, _NIT, body, 0)

    fence(final_sem)
    g0 = _NIT * GB
    nr = NU - g0 * NC
    pipe = Pipe(g0)
    pipe.restore(1)
    for k in range(1, nr + 1):
        qc = g0 * NC + k - ((NG - 1) * NC - 3)
        first = 0 if k == 1 else qc
        pre = [functools.partial(qblock, cc * R, (cc + 1) * R, (NG - 1) * GW, NG * GW)
               for cc in range(max(first, 0), min(qc + 1, NC))]
        pipe.step(k, nr, pre)
    for d in outs:
        d.wait()


def _dma_groups(H, NG, GB):
    groups = []
    pr, pc = 0, 0
    for (r1, c1) in _STAGES:
        grp = []
        if c1 > pc:
            grp.append(('wq', (pc, c1)))
        if r1 > pr:
            grp.append(('x', (pr, r1)))
        groups.append(grp)
        pr, pc = r1, c1
    groups[-1] += [('xt', 0), ('wqt', 0), ('k', 0), ('v', 0)]
    for i in range(_NIT):
        groups.append([(n, GB * i + 1 + j) for j in range(GB) for n in ('k', 'v')]
                      + [('wot', GB * i + j) for j in range(GB)])
    done = {key for grp in groups for key in grp}
    rest = [('wq', (pc, H * 128))] + [(n, g) for g in range(NG) for n in ('k', 'v', 'wot')]
    groups.append([key for key in rest if key not in done])
    return groups


@jax.jit
def pallas_standalone__mha_block_cached__near_ridge_kernel(x, k_cache, v_cache, wq, wo):
    B, Sq, D = x.shape
    _, H, Sk, Dh = k_cache.shape
    assert (B, Sq, D, H, Sk, Dh) == (16, 64, 576, 32, 64, 128)
    M = B * Sq
    DM = (D // 128) * 128
    NG = H // _G
    GB = _BODY // (B // 2 // _CH)
    bf, u32, f32 = jnp.bfloat16, jnp.uint32, jnp.float32
    ntl = _CH * _G
    nsem = len(_dma_groups(H, NG, GB)) + 1
    kernel = functools.partial(_mha_kernel, H=H, NP=B // 2, scale=Dh ** -0.5)
    out = pl.pallas_call(
        kernel,
        in_specs=[pl.BlockSpec(memory_space=pl.ANY)] * 5,
        out_specs=pl.BlockSpec(memory_space=pl.ANY),
        out_shape=jax.ShapeDtypeStruct((M, D), x.dtype),
        scratch_shapes=[
            pltpu.VMEM((M, D), bf),
            pltpu.VMEM((B, H, Sk, Dh), bf),
            pltpu.VMEM((B, H, Sk, Dh), bf),
            pltpu.VMEM((D, H * Dh), bf),
            pltpu.VMEM((D, H * Dh), bf),
            pltpu.VMEM((M // 2, H * Dh), u32),
            pltpu.VMEM((M // 2, GB * _G * Dh), u32),
            pltpu.VMEM((M // 2, 128), u32),
            pltpu.VMEM((ntl, 64, 128), f32),
            pltpu.VMEM((ntl, 32, 128), u32),
            pltpu.VMEM((ntl, 64, 128), f32),
            pltpu.VMEM((M, DM), f32),
            pltpu.VMEM((D - DM, M), f32),
            pltpu.VMEM((M, D), bf),
            pltpu.SemaphoreType.DMA((nsem,)),
        ],
        compiler_params=pltpu.CompilerParams(vmem_limit_bytes=100 * 1024 * 1024),
    )(x.reshape(M, D), k_cache, v_cache, wq, wo.T)
    return out.reshape(B, Sq, D)
```

```python
import functools

import jax
import jax.numpy as jnp
import jax.experimental.pallas as pl
import jax.experimental.pallas.tpu as pltpu

_LOG2E = 1.4426950408889634
_NT = (((1,), (1,)), ((), ()))
_TN = (((0,), (0,)), ((), ()))

_G = 4
_CH = 2
_BODY = 12
_NIT = 2
_KC = 1280
_STAGES = (
    ([(0, 512, 0, 128)], [(0, 128, 0, 512)], [(0, 512, 0, 512, 0, 128)]),
    ([(512, 1024, 0, 128)], [(0, 128, 512, _KC)],
     [(512, 1024, 0, _KC, 0, 128), (0, 512, 512, _KC, 0, 128)]),
    ([(0, 1024, 128, 384)], [(128, 384, 0, _KC)], [(0, 1024, 0, _KC, 128, 384)]),
    ([(0, 1024, 384, 512)], [(384, 512, 0, _KC), (0, 512, _KC, 2816)],
     [(0, 1024, 0, _KC, 384, 512), (0, 1024, _KC, 2816, 0, 512)]),
    ([], [(0, 512, 2816, 3584)], [(0, 1024, 2816, 3584, 0, 512)]),
)
_ORDER = ("s3,T1,m3,p3,p4,m2,s0,t0,p1,T0,s2,p7,p6,x2,m0,s1,x3,x4,p2,x7,x6,x0,p0,x1,t1,m1,p5,x5"
          ).split(",")
_ORDER_END = "m0,p0,p1,p2,p3,m1,p4,p5,p6,p7,t0,m2,t1,m3".split(",")


def _ld(ref, r0, r1, cs):
    return pltpu.bitcast(ref[r0 // 2:r1 // 2, cs], jnp.bfloat16)


def _st(ref, r0, r1, cs, val):
    ref[r0 // 2:r1 // 2, cs] = pltpu.bitcast(val, jnp.uint32)


def _lo_mask():
    return jax.lax.broadcasted_iota(jnp.int32, (64, 128), 1) < 64


def _softmax_cols(t, c):
    m = jnp.max(t, axis=0, keepdims=True)
    e = jnp.exp2((t - m) * c)
    l = jnp.sum(e, axis=0, keepdims=True)
    return e * (1.0 / l)


def _mha_kernel(x_hbm, k_hbm, v_hbm, wq_hbm, wot_hbm, out_hbm,
                x_v, k_v, v_v, wq_v, wot_v, q_scr, qp_scr, o_scr, w2_scr, sd_c, m2_c, pn_c,
                acc_scr, acct_scr, out_v, sems, *, H, NP, scale):
    G, CH = _G, _CH
    c = scale * _LOG2E
    R = CH * 128
    NC = NP // CH
    NG = H // G
    NU = NG * NC
    GW = G * 128
    D = out_v.shape[1]
    DM = (D // 128) * 128
    GB = _BODY // NC

    groups = _dma_groups(H, NG, GB)
    loop_sem0 = len(_STAGES)
    final_sem = len(groups) - 1
    out_sem = len(groups)
    sem_of = {key: i for i, grp in enumerate(groups) for key in grp}

    def dsl(i, w):
        if isinstance(i, int):
            return slice(i * w, (i + 1) * w)
        return pl.ds(pl.multiple_of(i * w, w), w)

    def cp(key, sem=None):
        kind, i = key
        if kind == 'out':
            return pltpu.make_async_copy(out_v.at[i[0]:i[1], :], out_hbm.at[i[0]:i[1], :], sems.at[out_sem])
        if sem is None:
            sem = sems.at[sem_of[key]]
        if kind == 'x':
            src, dst, sl = x_hbm, x_v, (slice(i[0], i[1]), slice(i[2], i[3]))
        elif kind == 'xt':
            src, dst, sl = x_hbm, x_v, (slice(None), slice(DM, D))
        elif kind == 'wq':
            src, dst, sl = wq_hbm, wq_v, (slice(i[0], i[1]), slice(i[2], i[3]))
        elif kind == 'wqt':
            src, dst, sl = wq_hbm, wq_v, (slice(DM, D), slice(None))
        elif kind == 'wot':
            src, dst, sl = wot_hbm, wot_v, (slice(None), dsl(i, GW))
        else:
            src, dst = (k_hbm, k_v) if kind == 'k' else (v_hbm, v_v)
            sl = (slice(None), dsl(i, G))
        return pltpu.make_async_copy(src.at[sl], dst.at[sl], sem)

    def fence(i):
        for key in groups[i]:
            cp(key).wait()

    def cols(g, w=GW, extra=0):
        if isinstance(g, int):
            return slice(g * GW + extra, g * GW + extra + w)
        return pl.ds(pl.multiple_of(g * GW + extra, 128), w)

    outs = []

    def qblock(r0, r1, c0, c1, k0=0, k1=DM):
        q = jnp.dot(x_v[r0:r1, k0:k1], wq_v[k0:k1, c0:c1], preferred_element_type=jnp.float32)
        if k0 > 0:
            q = q + qp_scr[r0:r1, c0:c1]
        if k1 < DM:
            qp_scr[r0:r1, c0:c1] = q
        else:
            _st(q_scr, r0, r1, slice(c0, c1), q.astype(jnp.bfloat16))

    def qblocks(r0, r1, c0, c1, k0=0, k1=DM):
        return [functools.partial(qblock, ra, min(ra + R, r1), ca, min(ca + GW, c1), k0, k1)
                for ca in range(c0, c1, GW) for ra in range(r0, r1, R)]

    def build_w2():
        for p in range(NP):
            xt = x_v[p * 128:(p + 1) * 128, DM:D]
            z = jnp.zeros((64, 64), xt.dtype)
            top = jnp.concatenate([z, xt[:64]], axis=1)
            bot = jnp.concatenate([xt[64:], z], axis=1)
            _st(w2_scr, p * 128, (p + 1) * 128, slice(None), jnp.concatenate([top, bot], axis=0))

    class Pipe:
        def __init__(self, gb):
            self.gb = gb
            self.sd, self.m2, self.tt, self.pn = {}, {}, {}, {}

        def grp(self, r):
            return self.gb + r // NC

        def tiles(self, r):
            ci = r % NC
            return [(r, p, h) for p in range(ci * CH, (ci + 1) * CH) for h in range(G)]

        def s_tile(self, r, p, h):
            g = self.grp(r)
            lo = _lo_mask()
            hc = cols(g, 128, h * 128)
            q1 = _ld(q_scr, p * 128, p * 128 + 64, hc)
            q2 = _ld(q_scr, p * 128 + 64, (p + 1) * 128, hc)
            wt = wq_v[DM:D, hc]
            k1 = k_v[2 * p, g * G + h]
            k2 = k_v[2 * p + 1, g * G + h]
            oa = jax.lax.dot_general(k1, jnp.concatenate([q1, wt], axis=0), _NT,
                                     preferred_element_type=jnp.float32)
            ob = jax.lax.dot_general(k2, jnp.concatenate([wt, q2], axis=0), _NT,
                                     preferred_element_type=jnp.float32)
            self.sd[r, p, h] = jnp.where(lo, oa, ob)
            self.m2[r, p, h] = jnp.where(lo, ob, oa).astype(jnp.bfloat16)

        def t_mm(self, r, pi):
            p = (r % NC) * CH + pi
            mc = jnp.concatenate([self.m2.pop((r, p, h)) for h in range(G)], axis=0)
            t = jax.lax.dot_general(mc, _ld(w2_scr, p * 128, (p + 1) * 128, slice(None)), _NT,
                                    preferred_element_type=jnp.float32)
            for h in range(G):
                self.tt[r, p, h] = t[h * 64:(h + 1) * 64]

        def sm_tile(self, r, p, h):
            self.pn[r, p, h] = _softmax_cols(self.sd.pop((r, p, h)) + self.tt.pop((r, p, h)), c)

        def pv_tile(self, r, p, h):
            g = self.grp(r)
            lo = _lo_mask()
            pn = self.pn.pop((r, p, h))
            z = jnp.zeros_like(pn)
            pt = jnp.concatenate([jnp.where(lo, pn, z), jnp.where(lo, z, pn)], axis=0).astype(jnp.bfloat16)
            vt = v_v[2 * p:2 * p + 2, g * G + h].reshape(128, 128)
            o = jax.lax.dot_general(pt, vt, _TN, preferred_element_type=jnp.float32)
            slot = (r // NC) % GB
            _st(o_scr, p * 128, (p + 1) * 128, cols(slot, 128, h * 128), o.astype(jnp.bfloat16))

        def o_parts(self, r, r0, r1):
            g = self.grp(r)
            final = isinstance(g, int) and g == NG - 1
            slot = (r // NC) % GB
            rows = slice(r0, r1)

            def main(n):
                nc = slice(n * 128, (n + 1) * 128)
                m = jax.lax.dot_general(_ld(o_scr, r0, r1, cols(slot)), wot_v[nc, cols(g)], _NT,
                                        preferred_element_type=jnp.float32)
                if final:
                    out_v[rows, nc] = (acc_scr[rows, nc] + m).astype(jnp.bfloat16)
                else:
                    acc_scr[rows, nc] += m

            def tail(pi):
                a, b = r0 + pi * 128, r0 + (pi + 1) * 128
                t = jax.lax.dot_general(wot_v[DM:D, cols(g)], _ld(o_scr, a, b, cols(slot)), _NT,
                                        preferred_element_type=jnp.float32)
                if final:
                    out_v[a:b, DM:D] = (acct_scr[:, a:b] + t).T.astype(jnp.bfloat16)
                else:
                    acct_scr[:, a:b] += t

            def write_out():
                d = cp(('out', (r0, r1)))
                d.start()
                outs.append(d)

            mains = [functools.partial(main, n) for n in range(DM // 128)]
            tails = [functools.partial(tail, i) for i in range((r1 - r0) // 128)]
            return mains, tails, (write_out if final else None)

        def prologue(self, fill):
            fill = list(fill)

            def f():
                if fill:
                    fill.pop(0)()

            for u in (0, 1):
                for tl in self.tiles(u):
                    self.s_tile(*tl)
                f()
            for u in (0, 1):
                for pi in range(CH):
                    self.t_mm(u, pi)
                for tl in self.tiles(u):
                    self.sm_tile(*tl)
                f()
                if u == 0:
                    for tl in self.tiles(2):
                        self.s_tile(*tl)
                    f()
            for tl in self.tiles(0):
                self.pv_tile(*tl)
            while fill:
                f()

        def step(self, k, nr, pre=()):
            for f in pre:
                f()
            ci = (k - 1) % NC
            g = self.grp(k - 1)
            if isinstance(g, int) and g == NG - 1 and ci == NC - 1:
                for r0 in range(ci * R, (ci + 1) * R, 128):
                    mains, tails, write_out = self.o_parts(k - 1, r0, r0 + 128)
                    for f in tails + mains:
                        f()
                    write_out()
                return
            mains, tails, write_out = self.o_parts(k - 1, ci * R, (ci + 1) * R)
            omap = {f'm{i}': m for i, m in enumerate(mains)}
            omap.update({f't{i}': t for i, t in enumerate(tails)})
            left = len(omap)
            for tok in (_ORDER if k + 1 < nr else _ORDER_END):
                i = int(tok[1:])
                if tok in omap:
                    omap[tok]()
                    left -= 1
                    if left == 0 and write_out is not None:
                        write_out()
                elif tok[0] == 's' and k + 2 < nr:
                    for tl in self.tiles(k + 2)[2 * i:2 * i + 2]:
                        self.s_tile(*tl)
                elif tok[0] == 'T' and k + 1 < nr:
                    self.t_mm(k + 1, i)
                elif tok[0] == 'x' and k + 1 < nr:
                    self.sm_tile(*self.tiles(k + 1)[i])
                elif tok[0] == 'p' and k < nr:
                    self.pv_tile(*self.tiles(k)[i])

        def save(self, k):
            for i, tl in enumerate(self.tiles(k + 1)):
                sd_c[i] = self.sd.pop(tl)
                m2_c[i] = pltpu.bitcast(self.m2.pop(tl), jnp.uint32)
            for i, tl in enumerate(self.tiles(k)):
                pn_c[i] = self.pn.pop(tl)

        def restore(self, k):
            for i, tl in enumerate(self.tiles(k + 1)):
                self.sd[tl] = sd_c[i]
                self.m2[tl] = pltpu.bitcast(m2_c[i], jnp.bfloat16)
            for i, tl in enumerate(self.tiles(k)):
                self.pn[tl] = pn_c[i]

    for grp in groups:
        for key in grp:
            cp(key).start()
    acc_scr[...] = jnp.zeros_like(acc_scr)
    acct_scr[...] = jnp.zeros_like(acct_scr)

    for si, (_, _, cbs) in enumerate(_STAGES):
        fence(si)
        qs = [f for cb in cbs for f in qblocks(*cb)]
        if si < len(_STAGES) - 1:
            for f in qs:
                f()
    build_w2()
    nfill = 6
    for f in qs[:-nfill]:
        f()
    pipe = Pipe(0)
    pipe.prologue(qs[-nfill:])
    pipe.save(1)

    def body(i, carry):
        for kind, gi in groups[loop_sem0]:
            cp((kind, gi + i * GB), sems.at[loop_sem0 + i]).wait()
        p = Pipe(i * GB)
        p.restore(1)
        for k in range(1, _BODY + 1):
            p.step(k, NU + 2)
        p.save(_BODY + 1)
        return carry

    jax.lax.fori_loop(0, _NIT, body, 0)

    fence(final_sem)
    g0 = _NIT * GB
    nr = NU - g0 * NC
    pipe = Pipe(g0)
    pipe.restore(1)
    for k in range(1, nr + 1):
        qc = g0 * NC + k - ((NG - 1) * NC - 3)
        first = 0 if k == 1 else qc
        pre = [functools.partial(qblock, cc * R, (cc + 1) * R, (NG - 1) * GW, NG * GW)
               for cc in range(max(first, 0), min(qc + 1, NC))]
        pipe.step(k, nr, pre)
    for d in outs:
        d.wait()


def _dma_groups(H, NG, GB):
    groups = []
    for (xs, ws, _) in _STAGES:
        groups.append([('wq', w) for w in ws] + [('x', x) for x in xs])
    pc = _STAGES[-1][1][-1][3]
    groups[-1] += [('xt', 0), ('wqt', 0), ('k', 0), ('v', 0)]
    for i in range(_NIT):
        groups.append([(n, GB * i + 1 + j) for j in range(GB) for n in ('k', 'v')]
                      + [('wot', GB * i + j) for j in range(GB)])
    done = {key for grp in groups for key in grp}
    rest = [('wq', (0, 512, pc, H * 128))] + [(n, g) for g in range(NG) for n in ('k', 'v', 'wot')]
    groups.append([key for key in rest if key not in done])
    return groups


@jax.jit
def pallas_standalone__mha_block_cached__near_ridge_kernel(x, k_cache, v_cache, wq, wo):
    B, Sq, D = x.shape
    _, H, Sk, Dh = k_cache.shape
    assert (B, Sq, D, H, Sk, Dh) == (16, 64, 576, 32, 64, 128)
    M = B * Sq
    DM = (D // 128) * 128
    NG = H // _G
    GB = _BODY // (B // 2 // _CH)
    bf, u32, f32 = jnp.bfloat16, jnp.uint32, jnp.float32
    ntl = _CH * _G
    nsem = len(_dma_groups(H, NG, GB)) + 1
    kernel = functools.partial(_mha_kernel, H=H, NP=B // 2, scale=Dh ** -0.5)
    out = pl.pallas_call(
        kernel,
        in_specs=[pl.BlockSpec(memory_space=pl.ANY)] * 5,
        out_specs=pl.BlockSpec(memory_space=pl.ANY),
        out_shape=jax.ShapeDtypeStruct((M, D), x.dtype),
        scratch_shapes=[
            pltpu.VMEM((M, D), bf),
            pltpu.VMEM((B, H, Sk, Dh), bf),
            pltpu.VMEM((B, H, Sk, Dh), bf),
            pltpu.VMEM((D, H * Dh), bf),
            pltpu.VMEM((D, H * Dh), bf),
            pltpu.VMEM((M // 2, H * Dh), u32),
            pltpu.VMEM((M, _KC), f32),
            pltpu.VMEM((M // 2, GB * _G * Dh), u32),
            pltpu.VMEM((M // 2, 128), u32),
            pltpu.VMEM((ntl, 64, 128), f32),
            pltpu.VMEM((ntl, 32, 128), u32),
            pltpu.VMEM((ntl, 64, 128), f32),
            pltpu.VMEM((M, DM), f32),
            pltpu.VMEM((D - DM, M), f32),
            pltpu.VMEM((M, D), bf),
            pltpu.SemaphoreType.DMA((nsem,)),
        ],
        compiler_params=pltpu.CompilerParams(vmem_limit_bytes=100 * 1024 * 1024),
    )(x.reshape(M, D), k_cache, v_cache, wq, wo.T)
    return out.reshape(B, Sq, D)
```

```python
import functools

import jax
import jax.numpy as jnp
import jax.experimental.pallas as pl
import jax.experimental.pallas.tpu as pltpu

_LOG2E = 1.4426950408889634
_NT = (((1,), (1,)), ((), ()))
_TN = (((0,), (0,)), ((), ()))

_G = 4
_CH = 2
_BODY = 12
_NIT = 2
_KC = 1280
_STAGES = (
    ([(0, 512, 0, 128)], [(0, 128, 0, 512)], [(0, 512, 0, 512, 0, 128)]),
    ([(512, 1024, 0, 128)], [(0, 128, 512, _KC)],
     [(512, 1024, 0, _KC, 0, 128), (0, 512, 512, _KC, 0, 128)]),
    ([(0, 1024, 128, 384)], [(128, 384, 0, _KC)], [(0, 1024, 0, _KC, 128, 384)]),
    ([(0, 1024, 384, 512)], [(384, 512, 0, _KC), (0, 512, _KC, 2816)],
     [(0, 1024, 0, _KC, 384, 512), (0, 1024, _KC, 2816, 0, 512)]),
    ([], [(0, 512, 2816, 3584)], [(0, 1024, 2816, 3584, 0, 512)]),
)
_ORDER = ("s3,T1,m3,p3,p4,m2,s0,t0,p1,T0,s2,p7,p6,x2,m0,s1,x3,x4,p2,x7,x6,x0,p0,x1,t1,m1,p5,x5"
          ).split(",")
_ORDER_END = "m0,p0,p1,p2,p3,m1,p4,p5,p6,p7,t0,m2,t1,m3".split(",")


def _ld(ref, r0, r1, cs):
    return pltpu.bitcast(ref[r0 // 2:r1 // 2, cs], jnp.bfloat16)


def _st(ref, r0, r1, cs, val):
    ref[r0 // 2:r1 // 2, cs] = pltpu.bitcast(val, jnp.uint32)


def _lo_mask():
    return jax.lax.broadcasted_iota(jnp.int32, (64, 128), 1) < 64


def _softmax_cols(t, c):
    m = jnp.max(t, axis=0, keepdims=True)
    e = jnp.exp2((t - m) * c)
    l = jnp.sum(e, axis=0, keepdims=True)
    return e * (1.0 / l)


def _mha_kernel(x_hbm, k_hbm, v_hbm, wq_hbm, wot_hbm, out_hbm,
                x_v, k_v, v_v, wq_v, wot_v, q_scr, qp_scr, o_scr, w2_scr, sd_c, m2_c, pn_c,
                acc_scr, acct_scr, out_v, sems, *, H, NP, scale):
    G, CH = _G, _CH
    c = scale * _LOG2E
    R = CH * 128
    NC = NP // CH
    NG = H // G
    NU = NG * NC
    GW = G * 128
    D = out_v.shape[1]
    DM = (D // 128) * 128
    GB = _BODY // NC

    groups = _dma_groups(H, NG, GB)
    loop_sem0 = len(_STAGES)
    final_sem = len(groups) - 1
    out_sem = len(groups)
    sem_of = {key: i for i, grp in enumerate(groups) for key in grp}

    def dsl(i, w):
        if isinstance(i, int):
            return slice(i * w, (i + 1) * w)
        return pl.ds(pl.multiple_of(i * w, w), w)

    def cp(key, sem=None):
        kind, i = key
        if kind == 'out':
            return pltpu.make_async_copy(out_v.at[i[0]:i[1], :], out_hbm.at[i[0]:i[1], :], sems.at[out_sem])
        if sem is None:
            sem = sems.at[sem_of[key]]
        if kind == 'x':
            src, dst, sl = x_hbm, x_v, (slice(i[0], i[1]), slice(i[2], i[3]))
        elif kind == 'xt':
            src, dst, sl = x_hbm, x_v, (slice(None), slice(DM, D))
        elif kind == 'wq':
            src, dst, sl = wq_hbm, wq_v, (slice(i[0], i[1]), slice(i[2], i[3]))
        elif kind == 'wqt':
            src, dst, sl = wq_hbm, wq_v, (slice(DM, D), slice(None))
        elif kind == 'wot':
            src, dst, sl = wot_hbm, wot_v, (slice(None), dsl(i, GW))
        elif kind in ('kc', 'vc'):
            src, dst = (k_hbm, k_v) if kind == 'kc' else (v_hbm, v_v)
            sl = (slice(i[1], i[2]), dsl(i[0], G))
        else:
            src, dst = (k_hbm, k_v) if kind == 'k' else (v_hbm, v_v)
            sl = (slice(None), dsl(i, G))
        return pltpu.make_async_copy(src.at[sl], dst.at[sl], sem)

    def fence(i):
        for key in groups[i]:
            cp(key).wait()

    def cols(g, w=GW, extra=0):
        if isinstance(g, int):
            return slice(g * GW + extra, g * GW + extra + w)
        return pl.ds(pl.multiple_of(g * GW + extra, 128), w)

    outs = []

    def qblock(r0, r1, c0, c1, k0=0, k1=DM):
        q = jnp.dot(x_v[r0:r1, k0:k1], wq_v[k0:k1, c0:c1], preferred_element_type=jnp.float32)
        if k0 > 0:
            q = q + qp_scr[r0:r1, c0:c1]
        if k1 < DM:
            qp_scr[r0:r1, c0:c1] = q
        else:
            _st(q_scr, r0, r1, slice(c0, c1), q.astype(jnp.bfloat16))

    def qblocks(r0, r1, c0, c1, k0=0, k1=DM):
        return [functools.partial(qblock, ra, min(ra + R, r1), ca, min(ca + GW, c1), k0, k1)
                for ca in range(c0, c1, GW) for ra in range(r0, r1, R)]

    def build_w2():
        for p in range(NP):
            xt = x_v[p * 128:(p + 1) * 128, DM:D]
            z = jnp.zeros((64, 64), xt.dtype)
            top = jnp.concatenate([z, xt[:64]], axis=1)
            bot = jnp.concatenate([xt[64:], z], axis=1)
            _st(w2_scr, p * 128, (p + 1) * 128, slice(None), jnp.concatenate([top, bot], axis=0))

    class Pipe:
        def __init__(self, gb):
            self.gb = gb
            self.sd, self.m2, self.tt, self.pn = {}, {}, {}, {}

        def grp(self, r):
            return self.gb + r // NC

        def tiles(self, r):
            ci = r % NC
            return [(r, p, h) for p in range(ci * CH, (ci + 1) * CH) for h in range(G)]

        def s_tile(self, r, p, h):
            g = self.grp(r)
            lo = _lo_mask()
            hc = cols(g, 128, h * 128)
            q1 = _ld(q_scr, p * 128, p * 128 + 64, hc)
            q2 = _ld(q_scr, p * 128 + 64, (p + 1) * 128, hc)
            wt = wq_v[DM:D, hc]
            k1 = k_v[2 * p, g * G + h]
            k2 = k_v[2 * p + 1, g * G + h]
            oa = jax.lax.dot_general(k1, jnp.concatenate([q1, wt], axis=0), _NT,
                                     preferred_element_type=jnp.float32)
            ob = jax.lax.dot_general(k2, jnp.concatenate([wt, q2], axis=0), _NT,
                                     preferred_element_type=jnp.float32)
            self.sd[r, p, h] = jnp.where(lo, oa, ob)
            self.m2[r, p, h] = jnp.where(lo, ob, oa).astype(jnp.bfloat16)

        def t_mm(self, r, pi):
            p = (r % NC) * CH + pi
            mc = jnp.concatenate([self.m2.pop((r, p, h)) for h in range(G)], axis=0)
            t = jax.lax.dot_general(mc, _ld(w2_scr, p * 128, (p + 1) * 128, slice(None)), _NT,
                                    preferred_element_type=jnp.float32)
            for h in range(G):
                self.tt[r, p, h] = t[h * 64:(h + 1) * 64]

        def sm_tile(self, r, p, h):
            self.pn[r, p, h] = _softmax_cols(self.sd.pop((r, p, h)) + self.tt.pop((r, p, h)), c)

        def pv_tile(self, r, p, h):
            g = self.grp(r)
            lo = _lo_mask()
            pn = self.pn.pop((r, p, h))
            z = jnp.zeros_like(pn)
            pt = jnp.concatenate([jnp.where(lo, pn, z), jnp.where(lo, z, pn)], axis=0).astype(jnp.bfloat16)
            vt = v_v[2 * p:2 * p + 2, g * G + h].reshape(128, 128)
            o = jax.lax.dot_general(pt, vt, _TN, preferred_element_type=jnp.float32)
            slot = (r // NC) % GB
            _st(o_scr, p * 128, (p + 1) * 128, cols(slot, 128, h * 128), o.astype(jnp.bfloat16))

        def o_parts(self, r, r0, r1):
            g = self.grp(r)
            final = isinstance(g, int) and g == NG - 1
            slot = (r // NC) % GB
            rows = slice(r0, r1)

            def main(n):
                nc = slice(n * 128, (n + 1) * 128)
                m = jax.lax.dot_general(_ld(o_scr, r0, r1, cols(slot)), wot_v[nc, cols(g)], _NT,
                                        preferred_element_type=jnp.float32)
                if final:
                    out_v[rows, nc] = (acc_scr[rows, nc] + m).astype(jnp.bfloat16)
                else:
                    acc_scr[rows, nc] += m

            def tail(pi):
                a, b = r0 + pi * 128, r0 + (pi + 1) * 128
                t = jax.lax.dot_general(wot_v[DM:D, cols(g)], _ld(o_scr, a, b, cols(slot)), _NT,
                                        preferred_element_type=jnp.float32)
                if final:
                    out_v[a:b, DM:D] = (acct_scr[:, a:b] + t).T.astype(jnp.bfloat16)
                else:
                    acct_scr[:, a:b] += t

            def write_out():
                d = cp(('out', (r0, r1)))
                d.start()
                outs.append(d)

            mains = [functools.partial(main, n) for n in range(DM // 128)]
            tails = [functools.partial(tail, i) for i in range((r1 - r0) // 128)]
            return mains, tails, (write_out if final else None)

        def prologue(self, fill):
            fill = list(fill)

            def f():
                if fill:
                    fill.pop(0)()

            for u in (0, 1):
                for tl in self.tiles(u):
                    self.s_tile(*tl)
                f()
            for u in (0, 1):
                for pi in range(CH):
                    self.t_mm(u, pi)
                for tl in self.tiles(u):
                    self.sm_tile(*tl)
                f()
                if u == 0:
                    for tl in self.tiles(2):
                        self.s_tile(*tl)
                    f()
            for tl in self.tiles(0):
                self.pv_tile(*tl)
            while fill:
                f()

        def step(self, k, nr, pre=()):
            for f in pre:
                f()
            ci = (k - 1) % NC
            g = self.grp(k - 1)
            if isinstance(g, int) and g == NG - 1 and ci == NC - 1:
                for r0 in range(ci * R, (ci + 1) * R, 128):
                    mains, tails, write_out = self.o_parts(k - 1, r0, r0 + 128)
                    for f in tails + mains:
                        f()
                    write_out()
                return
            mains, tails, write_out = self.o_parts(k - 1, ci * R, (ci + 1) * R)
            omap = {f'm{i}': m for i, m in enumerate(mains)}
            omap.update({f't{i}': t for i, t in enumerate(tails)})
            left = len(omap)
            for tok in (_ORDER if k + 1 < nr else _ORDER_END):
                i = int(tok[1:])
                if tok in omap:
                    omap[tok]()
                    left -= 1
                    if left == 0 and write_out is not None:
                        write_out()
                elif tok[0] == 's' and k + 2 < nr:
                    for tl in self.tiles(k + 2)[2 * i:2 * i + 2]:
                        self.s_tile(*tl)
                elif tok[0] == 'T' and k + 1 < nr:
                    self.t_mm(k + 1, i)
                elif tok[0] == 'x' and k + 1 < nr:
                    self.sm_tile(*self.tiles(k + 1)[i])
                elif tok[0] == 'p' and k < nr:
                    self.pv_tile(*self.tiles(k)[i])

        def save(self, k):
            for i, tl in enumerate(self.tiles(k + 1)):
                sd_c[i] = self.sd.pop(tl)
                m2_c[i] = pltpu.bitcast(self.m2.pop(tl), jnp.uint32)
            for i, tl in enumerate(self.tiles(k)):
                pn_c[i] = self.pn.pop(tl)

        def restore(self, k):
            for i, tl in enumerate(self.tiles(k + 1)):
                self.sd[tl] = sd_c[i]
                self.m2[tl] = pltpu.bitcast(m2_c[i], jnp.bfloat16)
            for i, tl in enumerate(self.tiles(k)):
                self.pn[tl] = pn_c[i]

    for grp in groups:
        for key in grp:
            cp(key).start()
    acc_scr[...] = jnp.zeros_like(acc_scr)
    acct_scr[...] = jnp.zeros_like(acct_scr)

    for si, (_, _, cbs) in enumerate(_STAGES):
        fence(si)
        qs = [f for cb in cbs for f in qblocks(*cb)]
        if si < len(_STAGES) - 1:
            for f in qs:
                f()
    build_w2()
    nfill = 6
    for f in qs[:-nfill]:
        f()
    pipe = Pipe(0)
    pipe.prologue(qs[-nfill:])
    pipe.save(1)

    def body(i, carry):
        for kind, gi in groups[loop_sem0]:
            key = (kind, (gi[0] + i * GB,) + gi[1:]) if isinstance(gi, tuple) else (kind, gi + i * GB)
            cp(key, sems.at[loop_sem0 + i]).wait()
        p = Pipe(i * GB)
        p.restore(1)
        for k in range(1, _BODY + 1):
            p.step(k, NU + 2)
        p.save(_BODY + 1)
        return carry

    jax.lax.fori_loop(0, _NIT, body, 0)

    fence(final_sem)
    g0 = _NIT * GB
    nr = NU - g0 * NC
    pipe = Pipe(g0)
    pipe.restore(1)
    for k in range(1, nr + 1):
        qc = g0 * NC + k - ((NG - 1) * NC - 3)
        first = 0 if k == 1 else qc
        pre = [functools.partial(qblock, cc * R, (cc + 1) * R, (NG - 1) * GW, NG * GW)
               for cc in range(max(first, 0), min(qc + 1, NC))]
        pipe.step(k, nr, pre)
    for d in outs:
        d.wait()


def _dma_groups(H, NG, GB):
    groups = []
    for (xs, ws, _) in _STAGES:
        groups.append([('wq', w) for w in ws] + [('x', x) for x in xs])
    pc = _STAGES[-1][1][-1][3]
    NB = 2 * _CH * (_BODY // GB)
    KS, VS = 3 * 2 * _CH, 2 * _CH
    groups[-1] += [('xt', 0), ('wqt', 0), ('kc', (0, 0, KS)), ('vc', (0, 0, VS))]
    for i in range(_NIT + 1):
        g0 = GB * i
        grp = [('kc', (g0, KS, NB)), ('vc', (g0, VS, NB))]
        if i < _NIT:
            grp += [(n, g0 + j) for j in range(1, GB) for n in ('k', 'v')]
            grp += [('kc', (g0 + GB, 0, KS)), ('vc', (g0 + GB, 0, VS))]
            grp += [('wot', g0 + j) for j in range(GB)]
        else:
            grp = [('wq', (0, 512, pc, H * 128))] + grp
            grp += [(n, g) for g in range(g0 + 1, NG) for n in ('k', 'v')]
            grp += [('wot', g) for g in range(g0, NG)]
        groups.append(grp)
    return groups


@jax.jit
def pallas_standalone__mha_block_cached__near_ridge_kernel(x, k_cache, v_cache, wq, wo):
    B, Sq, D = x.shape
    _, H, Sk, Dh = k_cache.shape
    assert (B, Sq, D, H, Sk, Dh) == (16, 64, 576, 32, 64, 128)
    M = B * Sq
    DM = (D // 128) * 128
    NG = H // _G
    GB = _BODY // (B // 2 // _CH)
    bf, u32, f32 = jnp.bfloat16, jnp.uint32, jnp.float32
    ntl = _CH * _G
    nsem = len(_dma_groups(H, NG, GB)) + 1
    kernel = functools.partial(_mha_kernel, H=H, NP=B // 2, scale=Dh ** -0.5)
    out = pl.pallas_call(
        kernel,
        in_specs=[pl.BlockSpec(memory_space=pl.ANY)] * 5,
        out_specs=pl.BlockSpec(memory_space=pl.ANY),
        out_shape=jax.ShapeDtypeStruct((M, D), x.dtype),
        scratch_shapes=[
            pltpu.VMEM((M, D), bf),
            pltpu.VMEM((B, H, Sk, Dh), bf),
            pltpu.VMEM((B, H, Sk, Dh), bf),
            pltpu.VMEM((D, H * Dh), bf),
            pltpu.VMEM((D, H * Dh), bf),
            pltpu.VMEM((M // 2, H * Dh), u32),
            pltpu.VMEM((M, _KC), f32),
            pltpu.VMEM((M // 2, GB * _G * Dh), u32),
            pltpu.VMEM((M // 2, 128), u32),
            pltpu.VMEM((ntl, 64, 128), f32),
            pltpu.VMEM((ntl, 32, 128), u32),
            pltpu.VMEM((ntl, 64, 128), f32),
            pltpu.VMEM((M, DM), f32),
            pltpu.VMEM((D - DM, M), f32),
            pltpu.VMEM((M, D), bf),
            pltpu.SemaphoreType.DMA((nsem,)),
        ],
        compiler_params=pltpu.CompilerParams(vmem_limit_bytes=100 * 1024 * 1024),
    )(x.reshape(M, D), k_cache, v_cache, wq, wo.T)
    return out.reshape(B, Sq, D)
```

```python
import functools

import jax
import jax.numpy as jnp
import jax.experimental.pallas as pl
import jax.experimental.pallas.tpu as pltpu

_LOG2E = 1.4426950408889634
_NT = (((1,), (1,)), ((), ()))
_TN = (((0,), (0,)), ((), ()))

_G = 4
_CH = 2
_BODY = 12
_NIT = 2
_KC = 3584
_STAGES = (
    ([(0, 512, 0, 128)], [(0, 128, 0, 768)], [(0, 512, 0, 768, 0, 128)]),
    ([(512, 1024, 0, 128)], [(0, 128, 768, 2048)],
     [(512, 1024, 0, 2048, 0, 128), (0, 512, 768, 2048, 0, 128)]),
    ([(0, 1024, 128, 256)], [(0, 128, 2048, _KC), (128, 256, 0, _KC)],
     [(0, 1024, 2048, _KC, 0, 128), (0, 1024, 0, _KC, 128, 256)]),
    ([(0, 1024, 256, 512)], [(256, 512, 0, _KC)], [(0, 1024, 0, _KC, 256, 512)]),
)
_ORDER = ("s1,T1,m3,p6,p3,m2,s0,t0,p1,T0,s3,p0,p4,x2,m0,s2,x3,x4,p2,p7,x6,x0,x7,x1,t1,m1,p5,x5"
          ).split(",")
_ORDER_END = "m0,p0,p1,p2,p3,m1,p4,p5,p6,p7,t0,m2,t1,m3".split(",")


def _ld(ref, r0, r1, cs):
    return pltpu.bitcast(ref[r0 // 2:r1 // 2, cs], jnp.bfloat16)


def _st(ref, r0, r1, cs, val):
    ref[r0 // 2:r1 // 2, cs] = pltpu.bitcast(val, jnp.uint32)


def _lo_mask():
    return jax.lax.broadcasted_iota(jnp.int32, (64, 128), 1) < 64


def _softmax_cols(t, c):
    m = jnp.max(t, axis=0, keepdims=True)
    e = jnp.exp2((t - m) * c)
    l = jnp.sum(e, axis=0, keepdims=True)
    return e * (1.0 / l)


def _mha_kernel(x_hbm, k_hbm, v_hbm, wq_hbm, wot_hbm, out_hbm,
                x_v, k_v, v_v, wq_v, wot_v, q_scr, qp_scr, o_scr, w2_scr, sd_c, m2_c, pn_c,
                acc_scr, acct_scr, out_v, sems, *, H, NP, scale):
    G, CH = _G, _CH
    c = scale * _LOG2E
    R = CH * 128
    NC = NP // CH
    NG = H // G
    NU = NG * NC
    GW = G * 128
    D = out_v.shape[1]
    DM = (D // 128) * 128
    GB = _BODY // NC

    groups = _dma_groups(H, NG, GB)
    loop_sem0 = len(_STAGES)
    final_sem = len(groups) - 1
    out_sem = len(groups)
    sem_of = {key: i for i, grp in enumerate(groups) for key in grp}

    def dsl(i, w):
        if isinstance(i, int):
            return slice(i * w, (i + 1) * w)
        return pl.ds(pl.multiple_of(i * w, w), w)

    def cp(key, sem=None):
        kind, i = key
        if kind == 'out':
            return pltpu.make_async_copy(out_v.at[i[0]:i[1], :], out_hbm.at[i[0]:i[1], :], sems.at[out_sem])
        if sem is None:
            sem = sems.at[sem_of[key]]
        if kind == 'x':
            src, dst, sl = x_hbm, x_v, (slice(i[0], i[1]), slice(i[2], i[3]))
        elif kind == 'xt':
            src, dst, sl = x_hbm, x_v, (slice(None), slice(DM, D))
        elif kind == 'wq':
            src, dst, sl = wq_hbm, wq_v, (slice(i[0], i[1]), slice(i[2], i[3]))
        elif kind == 'wqt':
            src, dst, sl = wq_hbm, wq_v, (slice(DM, D), slice(None))
        elif kind == 'wot':
            src, dst, sl = wot_hbm, wot_v, (slice(None), dsl(i, GW))
        elif kind in ('kc', 'vc'):
            src, dst = (k_hbm, k_v) if kind == 'kc' else (v_hbm, v_v)
            sl = (slice(i[1], i[2]), dsl(i[0], G))
        else:
            src, dst = (k_hbm, k_v) if kind == 'k' else (v_hbm, v_v)
            sl = (slice(None), dsl(i, G))
        return pltpu.make_async_copy(src.at[sl], dst.at[sl], sem)

    def fence(i):
        for key in groups[i]:
            cp(key).wait()

    def cols(g, w=GW, extra=0):
        if isinstance(g, int):
            return slice(g * GW + extra, g * GW + extra + w)
        return pl.ds(pl.multiple_of(g * GW + extra, 128), w)

    outs = []

    def qblock(r0, r1, c0, c1, k0=0, k1=DM):
        q = jnp.dot(x_v[r0:r1, k0:k1], wq_v[k0:k1, c0:c1], preferred_element_type=jnp.float32)
        if k0 > 0:
            q = q + qp_scr[r0:r1, c0:c1]
        if k1 < DM:
            qp_scr[r0:r1, c0:c1] = q
        else:
            _st(q_scr, r0, r1, slice(c0, c1), q.astype(jnp.bfloat16))

    def qblocks(r0, r1, c0, c1, k0=0, k1=DM):
        return [functools.partial(qblock, ra, min(ra + R, r1), ca, min(ca + GW, c1), k0, k1)
                for ca in range(c0, c1, GW) for ra in range(r0, r1, R)]

    def build_w2():
        for p in range(NP):
            xt = x_v[p * 128:(p + 1) * 128, DM:D]
            z = jnp.zeros((64, 64), xt.dtype)
            top = jnp.concatenate([z, xt[:64]], axis=1)
            bot = jnp.concatenate([xt[64:], z], axis=1)
            _st(w2_scr, p * 128, (p + 1) * 128, slice(None), jnp.concatenate([top, bot], axis=0))

    class Pipe:
        def __init__(self, gb):
            self.gb = gb
            self.sd, self.m2, self.tt, self.pn = {}, {}, {}, {}

        def grp(self, r):
            return self.gb + r // NC

        def tiles(self, r):
            ci = r % NC
            return [(r, p, h) for p in range(ci * CH, (ci + 1) * CH) for h in range(G)]

        def s_tile(self, r, p, h):
            g = self.grp(r)
            lo = _lo_mask()
            hc = cols(g, 128, h * 128)
            q1 = _ld(q_scr, p * 128, p * 128 + 64, hc)
            q2 = _ld(q_scr, p * 128 + 64, (p + 1) * 128, hc)
            wt = wq_v[DM:D, hc]
            k1 = k_v[2 * p, g * G + h]
            k2 = k_v[2 * p + 1, g * G + h]
            oa = jax.lax.dot_general(k1, jnp.concatenate([q1, wt], axis=0), _NT,
                                     preferred_element_type=jnp.float32)
            ob = jax.lax.dot_general(k2, jnp.concatenate([wt, q2], axis=0), _NT,
                                     preferred_element_type=jnp.float32)
            self.sd[r, p, h] = jnp.where(lo, oa, ob)
            self.m2[r, p, h] = jnp.where(lo, ob, oa).astype(jnp.bfloat16)

        def t_mm(self, r, pi):
            p = (r % NC) * CH + pi
            mc = jnp.concatenate([self.m2.pop((r, p, h)) for h in range(G)], axis=0)
            t = jax.lax.dot_general(mc, _ld(w2_scr, p * 128, (p + 1) * 128, slice(None)), _NT,
                                    preferred_element_type=jnp.float32)
            for h in range(G):
                self.tt[r, p, h] = t[h * 64:(h + 1) * 64]

        def sm_tile(self, r, p, h):
            self.pn[r, p, h] = _softmax_cols(self.sd.pop((r, p, h)) + self.tt.pop((r, p, h)), c)

        def pv_tile(self, r, p, h):
            g = self.grp(r)
            lo = _lo_mask()
            pn = self.pn.pop((r, p, h))
            z = jnp.zeros_like(pn)
            pt = jnp.concatenate([jnp.where(lo, pn, z), jnp.where(lo, z, pn)], axis=0).astype(jnp.bfloat16)
            vt = v_v[2 * p:2 * p + 2, g * G + h].reshape(128, 128)
            o = jax.lax.dot_general(pt, vt, _TN, preferred_element_type=jnp.float32)
            slot = (r // NC) % GB
            _st(o_scr, p * 128, (p + 1) * 128, cols(slot, 128, h * 128), o.astype(jnp.bfloat16))

        def o_parts(self, r, r0, r1):
            g = self.grp(r)
            final = isinstance(g, int) and g == NG - 1
            slot = (r // NC) % GB
            rows = slice(r0, r1)

            def main(n):
                nc = slice(n * 128, (n + 1) * 128)
                m = jax.lax.dot_general(_ld(o_scr, r0, r1, cols(slot)), wot_v[nc, cols(g)], _NT,
                                        preferred_element_type=jnp.float32)
                if final:
                    out_v[rows, nc] = (acc_scr[rows, nc] + m).astype(jnp.bfloat16)
                else:
                    acc_scr[rows, nc] += m

            def tail(pi):
                a, b = r0 + pi * 128, r0 + (pi + 1) * 128
                t = jax.lax.dot_general(wot_v[DM:D, cols(g)], _ld(o_scr, a, b, cols(slot)), _NT,
                                        preferred_element_type=jnp.float32)
                if final:
                    out_v[a:b, DM:D] = (acct_scr[:, a:b] + t).T.astype(jnp.bfloat16)
                else:
                    acct_scr[:, a:b] += t

            def write_out():
                d = cp(('out', (r0, r1)))
                d.start()
                outs.append(d)

            mains = [functools.partial(main, n) for n in range(DM // 128)]
            tails = [functools.partial(tail, i) for i in range((r1 - r0) // 128)]
            return mains, tails, (write_out if final else None)

        def prologue(self, fill):
            fill = list(fill)

            def f():
                if fill:
                    fill.pop(0)()

            for u in (0, 1):
                for tl in self.tiles(u):
                    self.s_tile(*tl)
                f()
            for u in (0, 1):
                for pi in range(CH):
                    self.t_mm(u, pi)
                for tl in self.tiles(u):
                    self.sm_tile(*tl)
                f()
                if u == 0:
                    for tl in self.tiles(2):
                        self.s_tile(*tl)
                    f()
            for tl in self.tiles(0):
                self.pv_tile(*tl)
            while fill:
                f()

        def step(self, k, nr, pre=()):
            for f in pre:
                f()
            ci = (k - 1) % NC
            g = self.grp(k - 1)
            if isinstance(g, int) and g == NG - 1 and ci == NC - 1:
                for r0 in range(ci * R, (ci + 1) * R, 128):
                    mains, tails, write_out = self.o_parts(k - 1, r0, r0 + 128)
                    for f in tails + mains:
                        f()
                    write_out()
                return
            mains, tails, write_out = self.o_parts(k - 1, ci * R, (ci + 1) * R)
            omap = {f'm{i}': m for i, m in enumerate(mains)}
            omap.update({f't{i}': t for i, t in enumerate(tails)})
            left = len(omap)
            for tok in (_ORDER if k + 1 < nr else _ORDER_END):
                i = int(tok[1:])
                if tok in omap:
                    omap[tok]()
                    left -= 1
                    if left == 0 and write_out is not None:
                        write_out()
                elif tok[0] == 's' and k + 2 < nr:
                    for tl in self.tiles(k + 2)[2 * i:2 * i + 2]:
                        self.s_tile(*tl)
                elif tok[0] == 'T' and k + 1 < nr:
                    self.t_mm(k + 1, i)
                elif tok[0] == 'x' and k + 1 < nr:
                    self.sm_tile(*self.tiles(k + 1)[i])
                elif tok[0] == 'p' and k < nr:
                    self.pv_tile(*self.tiles(k)[i])

        def save(self, k):
            for i, tl in enumerate(self.tiles(k + 1)):
                sd_c[i] = self.sd.pop(tl)
                m2_c[i] = pltpu.bitcast(self.m2.pop(tl), jnp.uint32)
            for i, tl in enumerate(self.tiles(k)):
                pn_c[i] = self.pn.pop(tl)

        def restore(self, k):
            for i, tl in enumerate(self.tiles(k + 1)):
                self.sd[tl] = sd_c[i]
                self.m2[tl] = pltpu.bitcast(m2_c[i], jnp.bfloat16)
            for i, tl in enumerate(self.tiles(k)):
                self.pn[tl] = pn_c[i]

    for grp in groups:
        for key in grp:
            cp(key).start()
    acc_scr[...] = jnp.zeros_like(acc_scr)
    acct_scr[...] = jnp.zeros_like(acct_scr)

    for si, (_, _, cbs) in enumerate(_STAGES):
        fence(si)
        qs = [f for cb in cbs for f in qblocks(*cb)]
        if si < len(_STAGES) - 1:
            for f in qs:
                f()
    build_w2()
    nfill = 6
    for f in qs[:-nfill]:
        f()
    pipe = Pipe(0)
    pipe.prologue(qs[-nfill:])
    pipe.save(1)

    def body(i, carry):
        for kind, gi in groups[loop_sem0]:
            key = (kind, (gi[0] + i * GB,) + gi[1:]) if isinstance(gi, tuple) else (kind, gi + i * GB)
            cp(key, sems.at[loop_sem0 + i]).wait()
        p = Pipe(i * GB)
        p.restore(1)
        for k in range(1, _BODY + 1):
            p.step(k, NU + 2)
        p.save(_BODY + 1)
        return carry

    jax.lax.fori_loop(0, _NIT, body, 0)

    fence(final_sem)
    g0 = _NIT * GB
    nr = NU - g0 * NC
    pipe = Pipe(g0)
    pipe.restore(1)
    for k in range(1, nr + 1):
        qc = g0 * NC + k - ((NG - 1) * NC - 3)
        first = 0 if k == 1 else qc
        pre = [functools.partial(qblock, cc * R, (cc + 1) * R, (NG - 1) * GW, NG * GW)
               for cc in range(max(first, 0), min(qc + 1, NC))]
        pipe.step(k, nr, pre)
    for d in outs:
        d.wait()


def _dma_groups(H, NG, GB):
    groups = []
    for (xs, ws, _) in _STAGES:
        groups.append([('wq', w) for w in ws] + [('x', x) for x in xs])
    pc = _KC
    NB = 2 * _CH * (_BODY // GB)
    KS, VS = 3 * 2 * _CH, 2 * _CH
    groups[-1] += [('xt', 0), ('wqt', 0), ('kc', (0, 0, KS)), ('vc', (0, 0, VS))]
    for i in range(_NIT + 1):
        g0 = GB * i
        grp = [('kc', (g0, KS, NB)), ('vc', (g0, VS, NB))]
        if i < _NIT:
            grp += [(n, g0 + j) for j in range(1, GB) for n in ('k', 'v')]
            grp += [('kc', (g0 + GB, 0, KS)), ('vc', (g0 + GB, 0, VS))]
            grp += [('wot', g0 + j) for j in range(GB)]
        else:
            grp = [('wq', (0, 512, pc, H * 128))] + grp
            grp += [(n, g) for g in range(g0 + 1, NG) for n in ('k', 'v')]
            grp += [('wot', g) for g in range(g0, NG)]
        groups.append(grp)
    return groups


@jax.jit
def pallas_standalone__mha_block_cached__near_ridge_kernel(x, k_cache, v_cache, wq, wo):
    B, Sq, D = x.shape
    _, H, Sk, Dh = k_cache.shape
    assert (B, Sq, D, H, Sk, Dh) == (16, 64, 576, 32, 64, 128)
    M = B * Sq
    DM = (D // 128) * 128
    NG = H // _G
    GB = _BODY // (B // 2 // _CH)
    bf, u32, f32 = jnp.bfloat16, jnp.uint32, jnp.float32
    ntl = _CH * _G
    nsem = len(_dma_groups(H, NG, GB)) + 1
    kernel = functools.partial(_mha_kernel, H=H, NP=B // 2, scale=Dh ** -0.5)
    out = pl.pallas_call(
        kernel,
        in_specs=[pl.BlockSpec(memory_space=pl.ANY)] * 5,
        out_specs=pl.BlockSpec(memory_space=pl.ANY),
        out_shape=jax.ShapeDtypeStruct((M, D), x.dtype),
        scratch_shapes=[
            pltpu.VMEM((M, D), bf),
            pltpu.VMEM((B, H, Sk, Dh), bf),
            pltpu.VMEM((B, H, Sk, Dh), bf),
            pltpu.VMEM((D, H * Dh), bf),
            pltpu.VMEM((D, H * Dh), bf),
            pltpu.VMEM((M // 2, H * Dh), u32),
            pltpu.VMEM((M, _KC), f32),
            pltpu.VMEM((M // 2, GB * _G * Dh), u32),
            pltpu.VMEM((M // 2, 128), u32),
            pltpu.VMEM((ntl, 64, 128), f32),
            pltpu.VMEM((ntl, 32, 128), u32),
            pltpu.VMEM((ntl, 64, 128), f32),
            pltpu.VMEM((M, DM), f32),
            pltpu.VMEM((D - DM, M), f32),
            pltpu.VMEM((M, D), bf),
            pltpu.SemaphoreType.DMA((nsem,)),
        ],
        compiler_params=pltpu.CompilerParams(vmem_limit_bytes=100 * 1024 * 1024),
    )(x.reshape(M, D), k_cache, v_cache, wq, wo.T)
    return out.reshape(B, Sq, D)
```
